```python
import jax
import jax.numpy as jnp

def _softmax(x, axis=-1):
    return jax.nn.softmax(x, axis=axis)
def _gelu(x):
    return jax.nn.gelu(x, approximate=True)
def _silu(x):
    return jax.nn.silu(x)
def _sigmoid(x):
    return jax.nn.sigmoid(x)
def _layernorm(x, axis=-1, eps=1e-5):
    m = jnp.mean(x, axis=axis, keepdims=True)
    v = jnp.var(x, axis=axis, keepdims=True)
    return (x - m) / jnp.sqrt(v + eps)
def _scatter_add(tgt, idx, src, axis=0):
    return tgt.at[idx].add(src)
def _segment_sum(src, seg, n):
    return jax.ops.segment_sum(src, seg, n)
class _Rng:
    def __init__(self, key):
        self._k = key
    def _next(self):
        self._k, sub = jax.random.split(self._k)
        return sub
    def normal(self, shape):
        return jax.random.normal(self._next(), shape, dtype=jnp.bfloat16)
    def randint(self, lo, hi, shape):
        return jax.random.randint(self._next(), shape, lo, hi, dtype=jnp.int32)
    def uniform(self, shape, lo=0.0, hi=1.0):
        return jax.random.uniform(self._next(), shape, jnp.bfloat16, lo, hi)
    def permutation(self, n):
        return jax.random.permutation(self._next(), n)


kernel_name = 'concat_heads__compressed_kv_cla__mha_block_cached__decode'

def setup_inputs():
    _rng = _Rng(jax.random.key(int.from_bytes(__import__("os").urandom(4), "little")))
    _w = (lambda a: (lambda t: t.astype(jnp.bfloat16) if jnp.issubdtype(t.dtype, jnp.floating) else t)(jnp.asarray(a)))
    def _A_setup():
        B, H, Sq, Sk, D, M = 4, 32, 1, 4096, 128, 512
        Dc = 4 * D
        return {
            "x": _w((lambda *s: _rng.normal(s) * 0.05)(B, Sq, M)),
            "c_kv": _w((lambda *s: _rng.normal(s) * 0.05)(B, Sk, Dc)),
            "w_q": _w((lambda *s: _rng.normal(s) * 0.05)(M, H, D) * (M ** -0.5)),
            "w_uk": _w((lambda *s: _rng.normal(s) * 0.05)(Dc, H, D) * (Dc ** -0.5)),
            "w_uv": _w((lambda *s: _rng.normal(s) * 0.05)(Dc, H, D) * (Dc ** -0.5)),
            "w_o": _w((lambda *s: _rng.normal(s) * 0.05)(H, D, M) * ((H * D) ** -0.5)),
        }
    _A_in = _A_setup()

    def _B_setup():
        B, Sq, D = 4, 1, 512
        H, Sk, Dh = 32, 4096, 128
        return {
            "x": _w((lambda *s: _rng.normal(s) * 0.05)(B, Sq, D)),
            "k_cache": _w((lambda *s: _rng.normal(s) * 0.05)(B, H, Sk, Dh)),
            "v_cache": _w((lambda *s: _rng.normal(s) * 0.05)(B, H, Sk, Dh)),
            "wq": _w((lambda *s: _rng.normal(s) * 0.05)(D, H * Dh) * (D ** -0.5)),
            "wo": _w((lambda *s: _rng.normal(s) * 0.05)(H * Dh, D) * ((H * Dh) ** -0.5)),
        }
    _B_in = _B_setup()

    return {
        "A_x": _A_in["x"],
        "A_c_kv": _A_in["c_kv"],
        "A_w_q": _A_in["w_q"],
        "A_w_uk": _A_in["w_uk"],
        "A_w_uv": _A_in["w_uv"],
        "A_w_o": _A_in["w_o"],
        "B_x": _B_in["x"],
        "B_k_cache": _B_in["k_cache"],
        "B_v_cache": _B_in["v_cache"],
        "B_wq": _B_in["wq"],
        "B_wo": _B_in["wo"],
    }

def reference(A_x, A_c_kv, A_w_q, A_w_uk, A_w_uv, A_w_o, B_x, B_k_cache, B_v_cache, B_wq, B_wo):
    def _A_ref(x, c_kv, w_q, w_uk, w_uv, w_o):
        B, Sq, M = x.shape[0], x.shape[1], x.shape[2]
        Sk = c_kv.shape[1]
        H, D = w_q.shape[1], w_q.shape[2]
        q = jnp.einsum("bqm,mhd->bhqd", x, w_q)
        k = jnp.einsum("bkc,chd->bhkd", c_kv, w_uk)
        v = jnp.einsum("bkc,chd->bhkd", c_kv, w_uv)
        scores = jnp.einsum("bhqd,bhkd->bhqk", q, k) * (D ** -0.5)
        off = Sk - Sq
        qi = jnp.arange(Sq)[:, None]
        kj = jnp.arange(Sk)[None, :]
        cmask = kj <= (qi + off)
        scores = jnp.where(cmask[None, None], scores, -1e9)
        p = _softmax(scores, axis=-1)
        ctx = jnp.einsum("bhqk,bhkd->bhqd", p, v)
        return jnp.einsum("bhqd,hdm->bqm", ctx, w_o)

    def _B_ref(x, k_cache, v_cache, wq, wo):
        B, Sq, D = x.shape
        H, Dh = 32, 128
        q = (lambda x, *d: x.transpose(*d))((x @ wq).reshape(B, Sq, H, Dh), 0, 2, 1, 3)
        scores = jnp.einsum("bhqd,bhkd->bhqk", q, k_cache) * (Dh ** -0.5)
        p = _softmax(scores, axis=-1)
        o = jnp.einsum("bhqk,bhkd->bhqd", p, v_cache)
        return (lambda x, *d: x.transpose(*d))(o, 0, 2, 1, 3).reshape(B, Sq, H * Dh) @ wo

    a = _A_ref(A_x, A_c_kv, A_w_q, A_w_uk, A_w_uv, A_w_o)
    b = _B_ref(B_x, B_k_cache, B_v_cache, B_wq, B_wo)
    return jnp.concatenate([a, b], axis=-1)
```

```python
import jax
import jax.numpy as jnp
from jax import lax
import jax.experimental.pallas as pl
import jax.experimental.pallas.tpu as pltpu

_B, _H, _D, _SK, _M, _DC = 4, 32, 128, 4096, 512, 512
_HG = 8
_NC = 8
_RC = _SK // _NC
_NG = _B * _H // _HG
_NSLOT = 4
_AHEAD = 2
_UNIT = 128
_SIDE = _UNIT // _NC
_KV = _RC // 16

_G_WOB, _G_WQA, _G_WUK, _G_C, _G_WUV, _G_WOA = 0, 1, 2, 3, 3 + _B, 4 + _B

_F32 = jnp.float32
_BF16 = jnp.bfloat16
_U32 = jnp.uint32


def _dot(a, b):
    return jnp.dot(a, b, preferred_element_type=_F32)


def _dot_nt(a, b):
    return lax.dot_general(a, b, (((1,), (1,)), ((), ())), preferred_element_type=_F32)


def _ds(start, size):
    return pl.ds(start if isinstance(start, int) else pl.multiple_of(start, size), size)


def _lane_tiles(x):
    return [x[:, t:t + 128] for t in range(0, x.shape[1], 128)]


def _kernel(xa_hbm, c_hbm, wqa_hbm, wuk_hbm, wuv_hbm, woa_hbm,
            xb_hbm, k_hbm, v_hbm, wqb_hbm, wob_hbm,
            o_ref,
            xa_buf, xb_buf, wqb_buf, wqa_buf, wuk_buf, wuv_buf, c_buf, woa_buf, wob_buf,
            kv_buf,
            qb_s, qa_s, qabs_s, ma_s, la_s, acca_s, cl_s, ctx_s, outa_s, outb_s,
            x_sem, wqb_sem, side_sem, k_sem, v_sem):
    scale = _D ** -0.5
    k_buf, v_buf = kv_buf.at[0], kv_buf.at[1]
    k_hbm, v_hbm, wqa_hbm, wuk_hbm, wuv_hbm = (
        r.bitcast(_U32) for r in (k_hbm, v_hbm, wqa_hbm, wuk_hbm, wuv_hbm))

    def start_side(src, dst, g, c):
        for t in range(_SIDE):
            rows = _ds((c * _SIDE + t) * 8, 8)
            pltpu.make_async_copy(src.at[:, rows], dst.at[:, rows],
                                  side_sem.at[g % 2]).start(priority=t % 2)

    def start_kv(step, j0, n):
        slot = step % _NSLOT
        heads = _ds((step // _NC) * _HG, _HG)
        for j in range(j0, j0 + n):
            src_rows = _ds((step % _NC) * (_RC // 2) + j * 8, 8)
            for hbm, buf, sem, queue in ((k_hbm, k_buf, k_sem, 0), (v_hbm, v_buf, v_sem, 1)):
                pltpu.make_async_copy(hbm.at[heads, src_rows], buf.at[slot, :, pl.ds(j * 8, 8)],
                                      sem.at[slot]).start(priority=queue)

    def wait_all(buf, sem):
        pltpu.make_async_copy(buf, buf, sem).wait()

    def head_pair(buf, j):
        words = buf[:, pl.ds(j, _M // 8, stride=_H // 2), :].reshape(_M, _D)
        even = lax.bitcast_convert_type(words << 16, _F32)
        odd = lax.bitcast_convert_type(words & jnp.uint32(0xFFFF0000), _F32)
        return even.astype(_BF16), odd.astype(_BF16)

    def rows8(x_buf):
        x = x_buf[...].astype(_F32)
        return jnp.concatenate([x, jnp.zeros_like(x)], axis=0).astype(_BF16)

    def wide_rows(buf, start, size):
        per_slab = buf.shape[1]
        return buf[start // per_slab, _ds(start % per_slab, size), :]

    pairs = _H // 2 // _NC

    def a_query(c):
        xa8 = rows8(xa_buf)
        for j in range(pairs):
            for i, w in enumerate(head_pair(wqa_buf, c * pairs + j)):
                qa_s[2 * (c * pairs + j) + i] = _dot(xa8, w)

    def a_absorb(c):
        for j in range(pairs):
            for i, w in enumerate(head_pair(wuk_buf, c * pairs + j)):
                h = 2 * (c * pairs + j) + i
                qabs = _dot_nt(qa_s[h].astype(_BF16), w)
                for b in range(_B):
                    qabs_s[b, pl.ds(h, 1), :] = qabs[b:b + 1]

    def a_attend(b, c):
        @pl.when(c == 0)
        def _():
            ma_s[...] = jnp.full(ma_s.shape, -jnp.inf, _F32)
            la_s[...] = jnp.zeros(la_s.shape, _F32)
            acca_s[...] = jnp.zeros(acca_s.shape, _F32)

        lat = wide_rows(c_buf.at[b], c * _RC, _RC)
        s = _dot_nt(qabs_s[b].astype(_BF16), lat) * scale
        m_old = ma_s[...]
        m_new = jnp.maximum(m_old, jnp.max(s, axis=1, keepdims=True))
        alpha = jnp.exp(m_old - m_new)
        p = jnp.exp(s - m_new[:, :1])
        ma_s[...] = m_new
        la_s[...] = alpha * la_s[...] + sum(_lane_tiles(p))
        acca_s[...] = alpha[:, :1] * acca_s[...] + _dot(p.astype(_BF16), lat)

        @pl.when(c == _NC - 1)
        def _():
            ctx = acca_s[...] / jnp.sum(la_s[...], axis=1, keepdims=True)
            for h in range(_H):
                cl_s[h, pl.ds(b, 1), :] = ctx[h:h + 1]

    def a_value(c):
        for j in range(pairs):
            for i, w in enumerate(head_pair(wuv_buf, c * pairs + j)):
                h = 2 * (c * pairs + j) + i
                ctx_s[h] = _dot(cl_s[h].astype(_BF16), w)

    def a_output(c):
        n = _H // _NC
        ctx = jnp.concatenate([ctx_s[c * n + i] for i in range(n)], axis=1)
        outa_s[...] += _dot(ctx.astype(_BF16), wide_rows(woa_buf, c * n * _D, n * _D))

    def side_work(g, c):
        fetch = ((_G_WOB, wob_hbm, wob_buf), (_G_WQA, wqa_hbm, wqa_buf), (_G_WUK, wuk_hbm, wuk_buf),
                 (_G_WUV, wuv_hbm, wuv_buf), (_G_WOA, woa_hbm, woa_buf))
        for g0, src, dst in fetch:
            pl.when(g == g0)(lambda: start_side(src, dst, g, c))

        @pl.when((g >= _G_C) & (g < _G_C + _B))
        def _():
            start_side(c_hbm.at[g - _G_C], c_buf.at[g - _G_C], g, c)

        def consume(buf, work):
            pl.when(c == 0)(lambda: wait_all(buf, side_sem.at[(g - 1) % 2]))
            work(c)

        use = ((_G_WQA, wqa_buf, a_query), (_G_WUK, wuk_buf, a_absorb),
               (_G_WUV, wuv_buf, a_value), (_G_WOA, woa_buf, a_output))
        for g0, buf, work in use:
            pl.when(g == g0 + 1)(lambda: consume(buf, work))

        @pl.when((g > _G_C) & (g <= _G_C + _B))
        def _():
            b = g - _G_C - 1
            consume(c_buf.at[b], lambda c: a_attend(b, c))

    def start_wqb(i):
        for t in range(16):
            rows, cols = _ds((i * 2 + t // 8) * 8, 8), pl.ds((t % 8) * 512, 512)
            pltpu.make_async_copy(wqb_hbm.at[:, rows, cols], wqb_buf.at[:, rows, cols],
                                  wqb_sem).start(priority=t % 2)

    xb_copy = pltpu.make_async_copy(xb_hbm, xb_buf, x_sem.at[0])
    xa_copy = pltpu.make_async_copy(xa_hbm, xa_buf, x_sem.at[1])
    start_wqb(0)
    xb_copy.start()
    xa_copy.start()
    pl.loop(1, _UNIT // 16)(start_wqb)
    for step in range(_AHEAD - 1):
        start_kv(step, 0, _KV)

    cl_s[...] = jnp.zeros(cl_s.shape, _F32)
    outa_s[...] = jnp.zeros(outa_s.shape, _F32)
    outb_s[...] = jnp.zeros(outb_s.shape, _F32)

    xb_copy.wait()
    xa_copy.wait()
    xb8 = rows8(xb_buf)
    wait_all(wqb_buf, wqb_sem)
    for h in range(_H):
        q = _dot(xb8, wqb_buf[:, :, h * _D:(h + 1) * _D].reshape(_M, _D))
        for b in range(_B):
            qb_s[pl.ds(b * _H + h, 1), :] = q[b:b + 1]
        start_kv(_AHEAD - 1, h * _KV // _H, _KV // _H)

    sub = lax.broadcasted_iota(jnp.int32, (_HG, _D), 0)
    sub_rc = lax.broadcasted_iota(jnp.int32, (_HG, _RC), 0)
    per_dot = _KV // (2 * _HG)

    def kv_step(g, c, q, carry, last_group, prefetch):
        m, l, acc = carry
        step = g * _NC + c
        slot = step % _NSLOT
        if not last_group:
            pl.when(g <= _G_WOA + 1)(lambda: side_work(g, c))
        wait_all(k_buf.at[slot], k_sem.at[slot])
        s = None
        for i in range(_HG):
            si = _dot_nt(q, pltpu.bitcast(k_buf[slot, i], _BF16))
            s = si if s is None else jnp.where(sub_rc == i, si, s)
            if prefetch:
                start_kv(step + _AHEAD, i * per_dot, per_dot)
        s = s * scale
        m_new = jnp.maximum(m, jnp.max(s, axis=1, keepdims=True))
        alpha = jnp.exp(m - m_new)
        p = jnp.exp(s - m_new)
        l = alpha * l + sum(_lane_tiles(p))
        p = p.astype(_BF16)
        wait_all(v_buf.at[slot], v_sem.at[slot])
        pv = None
        for i in range(_HG):
            pvi = _dot(p, pltpu.bitcast(v_buf[slot, i], _BF16))
            pv = pvi if pv is None else jnp.where(sub == i, pvi, pv)
            if prefetch:
                start_kv(step + _AHEAD, (_HG + i) * per_dot, per_dot)
        return m_new, l, alpha * acc + pv

    def group(g, last_group):
        q = qb_s[_ds(g * _HG, _HG), :].astype(_BF16)
        carry = (jnp.full((_HG, 1), -jnp.inf, _F32), jnp.zeros((_HG, _D), _F32),
                 jnp.zeros((_HG, _D), _F32))
        n_pre = _NC - _AHEAD if last_group else _NC
        carry = lax.fori_loop(
            0, n_pre, lambda c, x: kv_step(g, c, q, x, last_group, True), carry)
        if last_group:
            carry = lax.fori_loop(
                n_pre, _NC, lambda c, x: kv_step(g, c, q, x, True, False), carry)
        else:
            pl.when(g == _G_WOB)(lambda: wait_all(wob_buf, side_sem.at[_G_WOB % 2]))
        _, l, acc = carry
        o = acc / jnp.sum(l, axis=1, keepdims=True)
        o = jnp.concatenate([jnp.where(sub == i, o, 0.0) for i in range(_HG)], axis=1)
        w = wide_rows(wob_buf, (g % (_H // _HG)) * _HG * _D, _HG * _D)
        outb_s[g // (_H // _HG)] += _dot(o.astype(_BF16), w)

    pl.loop(0, _NG - 1)(lambda g: group(g, False))
    group(_NG - 1, True)

    out_b = jnp.concatenate(
        [jnp.sum(outb_s[b], axis=0, keepdims=True) for b in range(_B)], axis=0)
    o_ref[:, 0:_M] = outa_s[0:_B, :].astype(o_ref.dtype)
    o_ref[:, _M:2 * _M] = out_b.astype(o_ref.dtype)


@jax.jit
def pallas_concat_heads__compressed_kv_cla__mha_block_cached__decode_kernel(
    A_x: jax.Array,
    A_c_kv: jax.Array,
    A_w_q: jax.Array,
    A_w_uk: jax.Array,
    A_w_uv: jax.Array,
    A_w_o: jax.Array,
    B_x: jax.Array,
    B_k_cache: jax.Array,
    B_v_cache: jax.Array,
    B_wq: jax.Array,
    B_wo: jax.Array,
):
    assert A_x.shape == (_B, 1, _M) and A_c_kv.shape == (_B, _SK, _DC)
    assert A_w_q.shape == (_M, _H, _D) and B_k_cache.shape == (_B, _H, _SK, _D)
    head_w = (8, _M * _H // 8, _D)
    head_words = (8, _M * _H // 16, _D)
    wide_w = (4, _SK // 4, _DC)
    wqb_w = (4, _M // 4, _H * _D)
    kv_words = (2, _NSLOT, _HG, _RC // 2, _D)
    dma = pltpu.SemaphoreType.DMA
    out = pl.pallas_call(
        _kernel,
        in_specs=[pl.BlockSpec(memory_space=pl.ANY)] * 11,
        out_specs=pl.BlockSpec(memory_space=pltpu.VMEM),
        out_shape=jax.ShapeDtypeStruct((_B, 2 * _M), A_x.dtype),
        scratch_shapes=[
            pltpu.VMEM((_B, _M), _BF16),
            pltpu.VMEM((_B, _M), _BF16),
            pltpu.VMEM(wqb_w, _BF16),
            pltpu.VMEM(head_words, _U32),
            pltpu.VMEM(head_words, _U32),
            pltpu.VMEM(head_words, _U32),
            pltpu.VMEM((_B,) + wide_w, _BF16),
            pltpu.VMEM(wide_w, _BF16),
            pltpu.VMEM(wide_w, _BF16),
            pltpu.VMEM(kv_words, _U32),
            pltpu.VMEM((_B * _H, _D), _F32),
            pltpu.VMEM((_H, 8, _D), _F32),
            pltpu.VMEM((_B, _H, _DC), _F32),
            pltpu.VMEM((_H, 128), _F32),
            pltpu.VMEM((_H, 128), _F32),
            pltpu.VMEM((_H, _DC), _F32),
            pltpu.VMEM((_H, 8, _DC), _F32),
            pltpu.VMEM((_H, 8, _D), _F32),
            pltpu.VMEM((8, _M), _F32),
            pltpu.VMEM((_B, 8, _M), _F32),
            dma((2,)), dma(()), dma((2,)), dma((_NSLOT,)), dma((_NSLOT,)),
        ],
        compiler_params=pltpu.CompilerParams(
            vmem_limit_bytes=100 * 1024 * 1024, disable_bounds_checks=True),
    )(
        A_x.reshape(_B, _M),
        A_c_kv.reshape((_B,) + wide_w),
        A_w_q.reshape(head_w),
        A_w_uk.reshape(head_w),
        A_w_uv.reshape(head_w),
        A_w_o.reshape(wide_w),
        B_x.reshape(_B, _M),
        B_k_cache.reshape(_B * _H, _SK, _D),
        B_v_cache.reshape(_B * _H, _SK, _D),
        B_wq.reshape(wqb_w),
        B_wo.reshape(wide_w),
    )
    return out.reshape(_B, 1, 2 * _M)
```

```python
import jax
import jax.numpy as jnp
from jax import lax
import jax.experimental.pallas as pl
import jax.experimental.pallas.tpu as pltpu

_B, _H, _D, _SK, _M, _DC = 4, 32, 128, 4096, 512, 512
_HG = 8
_NC = 8
_RC = _SK // _NC
_NG = _B * _H // _HG
_NSLOT = 4
_AHEAD = 2
_KV = 32
_UNIT = 128
_SHARE = _UNIT // _NC

_F32 = jnp.float32
_BF16 = jnp.bfloat16
_U32 = jnp.uint32


def _dot(a, b):
    return jnp.dot(a, b, preferred_element_type=_F32)


def _dot_nt(a, b):
    return lax.dot_general(a, b, (((1,), (1,)), ((), ())), preferred_element_type=_F32)


def _ds(start, size):
    return pl.ds(start if isinstance(start, int) else pl.multiple_of(start, size), size)


def _lane_sum(x):
    return sum(x[:, t:t + 128] for t in range(0, x.shape[1], 128))


def _kernel(xa_hbm, c_hbm, wqa_hbm, wuk_hbm, wuv_hbm, woa_hbm,
            xb_hbm, k_hbm, v_hbm, wqb_hbm, wob_hbm,
            o_ref,
            xa_buf, c_buf, wqa_buf, wuk_buf, wuv_buf, woa_buf,
            xb_buf, kv_buf, wqb_buf, wob_buf,
            qa_s, qabs_s, ma_s, la_s, acca_s, cl_s, ctx_s, qb_s, outb_s,
            x_sem, c_sem, w_sem, woa_sem, k_sem, v_sem):
    scale = _D ** -0.5
    k_buf, v_buf = kv_buf.at[0], kv_buf.at[1]
    k_hbm, v_hbm, wqa_hbm, wuk_hbm, wuv_hbm = (
        r.bitcast(_U32) for r in (k_hbm, v_hbm, wqa_hbm, wuk_hbm, wuv_hbm))

    wqb, wob, wqa, wuk, wuv = (
        (src, dst, w_sem.at[i]) for i, (src, dst) in enumerate((
            (wqb_hbm, wqb_buf), (wob_hbm, wob_buf),
            (wqa_hbm, wqa_buf), (wuk_hbm, wuk_buf), (wuv_hbm, wuv_buf))))

    def latent(b):
        return c_hbm.at[b], c_buf.at[b], c_sem.at[b]

    def start_unit(unit, share, t, queue):
        src, dst, sem = unit
        n = src.shape[1] * 2 // _UNIT
        at = (pl.ds(t % 2 * 2, 2), _ds((share * (_SHARE // 2) + t // 2) * n, n))
        pltpu.make_async_copy(src.at[at], dst.at[at], sem).start(priority=queue)

    def start_kv(step, j):
        slot = step % _NSLOT
        head, row = j % 4 * 2, j // 4 * 32
        src = (_ds(step // _NC * _HG + head, 2), _ds(step % _NC * (_RC // 2) + row, 32))
        dst = (slot, pl.ds(head, 2), pl.ds(row, 32))
        pltpu.make_async_copy(k_hbm.at[src], k_buf.at[dst], k_sem.at[slot]).start(priority=1)
        pltpu.make_async_copy(v_hbm.at[src], v_buf.at[dst], v_sem.at[slot]).start(priority=0)

    def wait_all(buf, sem):
        pltpu.make_async_copy(buf, buf, sem).wait()

    def head_pair(buf, j):
        words = buf[:, pl.ds(j, _M // 4, stride=_H // 2), :].reshape(_M, _D)
        even = lax.bitcast_convert_type(words << 16, _F32)
        odd = lax.bitcast_convert_type(words & jnp.uint32(0xFFFF0000), _F32)
        return even.astype(_BF16), odd.astype(_BF16)

    def heads_of(buf, c):
        pairs = _H // 2 // _NC
        for j in range(pairs):
            for i, w in enumerate(head_pair(buf, c * pairs + j)):
                yield 2 * (c * pairs + j) + i, w

    def rows8(x_buf):
        x = x_buf[...].astype(_F32)
        return jnp.concatenate([x, jnp.zeros_like(x)], axis=0).astype(_BF16)

    def a_query(c):
        x = rows8(xa_buf)
        for h, w in heads_of(wqa_buf, c):
            qa_s[h] = _dot(x, w)

    def a_absorb(c):
        for h, w in heads_of(wuk_buf, c):
            qabs = _dot_nt(qa_s[h].astype(_BF16), w)
            for b in range(_B):
                qabs_s[b, pl.ds(h, 1), :] = qabs[b:b + 1]

    def a_attend(b, c):
        @pl.when(c == 0)
        def _():
            ma_s[...] = jnp.full(ma_s.shape, -jnp.inf, _F32)
            la_s[...] = jnp.zeros(la_s.shape, _F32)
            acca_s[...] = jnp.zeros(acca_s.shape, _F32)

        lat = c_buf[b, c // 2, _ds(c % 2 * _RC, _RC), :]
        s = _dot_nt(qabs_s[b].astype(_BF16), lat) * scale
        m_old = ma_s[...]
        m_new = jnp.maximum(m_old, jnp.max(s, axis=1, keepdims=True))
        alpha = jnp.exp(m_old - m_new)
        p = jnp.exp(s - m_new[:, :1])
        ma_s[...] = m_new
        la_s[...] = alpha * la_s[...] + _lane_sum(p)
        acca_s[...] = alpha[:, :1] * acca_s[...] + _dot(p.astype(_BF16), lat)

        @pl.when(c == _NC - 1)
        def _():
            ctx = acca_s[...] / jnp.sum(la_s[...], axis=1, keepdims=True)
            for h in range(_H):
                cl_s[h, pl.ds(b, 1), :] = ctx[h:h + 1]

    def a_value(c):
        for h, w in heads_of(wuv_buf, c):
            ctx_s[h] = _dot(cl_s[h].astype(_BF16), w)

    def a_output(c):
        share = woa_buf.at[:, pl.ds(c * _D, _D)]
        wait_all(share, woa_sem.at[c])
        ctx = jnp.concatenate([ctx_s[h] for h in range(c, _H, _NC)], axis=1)
        return _dot(ctx.astype(_BF16), share[...].reshape(_H // _NC * _D, _M))

    def side_work(g, c):
        def fetch(*units):
            for t in range(_SHARE):
                for queue, unit in enumerate(units):
                    start_unit(unit, c, t, queue)

        def consume(unit, work):
            pl.when(c == 0)(lambda: wait_all(*unit[1:]))
            work(c)

        pl.when(g == 0)(lambda: fetch(wob, wqa))
        pl.when(g == 1)(lambda: fetch(wuk, wuv))
        pl.when((g >= 2) & (g < 2 + _B // 2))(
            lambda: fetch(latent(g - 2), latent(g - 2 + _B // 2)))
        pl.when(g == 1)(lambda: consume(wqa, a_query))
        pl.when(g == 2)(lambda: consume(wuk, a_absorb))
        pl.when((g >= 3) & (g < 3 + _B))(
            lambda: consume(latent(g - 3), lambda c: a_attend(g - 3, c)))
        pl.when(g == 3 + _B)(lambda: consume(wuv, a_value))

    def start_wqb(i):
        for t in range(_SHARE):
            at = (pl.ds(t % 2 * 2, 2), _ds((i * 2 + t // 8) * 8, 8), pl.ds(t // 2 % 4 * 1024, 1024))
            pltpu.make_async_copy(wqb_hbm.at[at], wqb_buf.at[at], wqb[2]).start(priority=t % 2)

    xb_copy = pltpu.make_async_copy(xb_hbm, xb_buf, x_sem.at[0])
    xa_copy = pltpu.make_async_copy(xa_hbm, xa_buf, x_sem.at[1])
    start_wqb(0)
    xb_copy.start()
    xa_copy.start()
    pl.loop(1, _NC)(start_wqb)
    for step in range(_AHEAD - 1):
        for j in range(_KV):
            start_kv(step, j)

    cl_s[...] = jnp.zeros(cl_s.shape, _F32)
    outb_s[...] = jnp.zeros(outb_s.shape, _F32)

    xb_copy.wait()
    xa_copy.wait()
    xb = rows8(xb_buf)
    wait_all(*wqb[1:])
    for h in range(_H):
        q = _dot(xb, wqb_buf[:, :, h * _D:(h + 1) * _D].reshape(_M, _D))
        for b in range(_B):
            qb_s[pl.ds(b * _H + h, 1), :] = q[b:b + 1]
        start_kv(_AHEAD - 1, h)

    sub = lax.broadcasted_iota(jnp.int32, (_HG, _D), 0)
    sub_rc = lax.broadcasted_iota(jnp.int32, (_HG, _RC), 0)
    n_dot = 2 * _HG

    def request_kv(step):
        def request(i):
            for j in range(i * _KV // n_dot, (i + 1) * _KV // n_dot):
                start_kv(step, j)
        return request

    def request_woa(part):
        def request(i):
            n = _UNIT // (_AHEAD * n_dot)
            for j in range((part * n_dot + i) * n, (part * n_dot + i + 1) * n):
                share = j // _SHARE
                start_unit((woa_hbm, woa_buf, woa_sem.at[share]), share, j % _SHARE, j % 2)
        return request

    def kv_step(step, q, carry, request):
        m, l, acc = carry
        slot = step % _NSLOT
        wait_all(k_buf.at[slot], k_sem.at[slot])
        s = None
        for i in range(_HG):
            si = _dot_nt(q, pltpu.bitcast(k_buf[slot, i], _BF16))
            s = si if s is None else jnp.where(sub_rc == i, si, s)
            request(i)
        s = s * scale
        m_new = jnp.maximum(m, jnp.max(s, axis=1, keepdims=True))
        alpha = jnp.exp(m - m_new)
        p = jnp.exp(s - m_new)
        l = alpha * l + _lane_sum(p)
        p = p.astype(_BF16)
        wait_all(v_buf.at[slot], v_sem.at[slot])
        pv = None
        for i in range(_HG):
            pvi = _dot(p, pltpu.bitcast(v_buf[slot, i], _BF16))
            pv = pvi if pv is None else jnp.where(sub == i, pvi, pv)
            request(_HG + i)
        return m_new, l, alpha * acc + pv

    def group(g, last):
        q = qb_s[_ds(g * _HG, _HG), :].astype(_BF16)
        carry = (jnp.full((_HG, 1), -jnp.inf, _F32), jnp.zeros((_HG, _D), _F32),
                 jnp.zeros((_HG, _D), _F32))

        def body(c, carry):
            if not last:
                pl.when(g <= 3 + _B)(lambda: side_work(g, c))
            step = g * _NC + c
            return kv_step(step, q, carry, request_kv(step + _AHEAD))

        if last:
            carry = lax.fori_loop(0, _NC - _AHEAD, body, carry)
            for part in range(_AHEAD):
                carry = kv_step((g + 1) * _NC - _AHEAD + part, q, carry, request_woa(part))
        else:
            carry = lax.fori_loop(0, _NC, body, carry)
            pl.when(g == 0)(lambda: wait_all(*wob[1:]))
        _, l, acc = carry
        o = acc / jnp.sum(l, axis=1, keepdims=True)
        o = jnp.concatenate([jnp.where(sub == i, o, 0.0) for i in range(_HG)], axis=1)
        outb_s[g // (_H // _HG)] += _dot(o.astype(_BF16), wob_buf[g % (_H // _HG)])

    pl.loop(0, _NG - 1)(lambda g: group(g, False))
    group(_NG - 1, True)

    out_b = jnp.concatenate(
        [jnp.sum(outb_s[b], axis=0, keepdims=True) for b in range(_B)], axis=0)
    o_ref[:, _M:2 * _M] = out_b.astype(o_ref.dtype)
    out_a = sum(a_output(c) for c in range(_NC))
    o_ref[:, 0:_M] = out_a[0:_B].astype(o_ref.dtype)


@jax.jit
def pallas_concat_heads__compressed_kv_cla__mha_block_cached__decode_kernel(
    A_x: jax.Array,
    A_c_kv: jax.Array,
    A_w_q: jax.Array,
    A_w_uk: jax.Array,
    A_w_uv: jax.Array,
    A_w_o: jax.Array,
    B_x: jax.Array,
    B_k_cache: jax.Array,
    B_v_cache: jax.Array,
    B_wq: jax.Array,
    B_wo: jax.Array,
):
    assert A_x.shape == B_x.shape == (_B, 1, _M) and A_c_kv.shape == (_B, _SK, _DC)
    assert A_w_q.shape == (_M, _H, _D) and B_k_cache.shape == (_B, _H, _SK, _D)
    head_w = (4, _M * _H // 4, _D)
    head_words = (4, _M * _H // 8, _D)
    wide_w = (4, _SK // 4, _DC)
    wqb_w = (4, _M // 4, _H * _D)
    dma = pltpu.SemaphoreType.DMA
    out = pl.pallas_call(
        _kernel,
        in_specs=[pl.BlockSpec(memory_space=pl.ANY)] * 11,
        out_specs=pl.BlockSpec(memory_space=pltpu.VMEM),
        out_shape=jax.ShapeDtypeStruct((_B, 2 * _M), A_x.dtype),
        scratch_shapes=[
            pltpu.VMEM((_B, _M), _BF16),
            pltpu.VMEM((_B,) + wide_w, _BF16),
            pltpu.VMEM(head_words, _U32),
            pltpu.VMEM(head_words, _U32),
            pltpu.VMEM(head_words, _U32),
            pltpu.VMEM(wide_w, _BF16),
            pltpu.VMEM((_B, _M), _BF16),
            pltpu.VMEM((2, _NSLOT, _HG, _RC // 2, _D), _U32),
            pltpu.VMEM(wqb_w, _BF16),
            pltpu.VMEM(wide_w, _BF16),
            pltpu.VMEM((_H, 8, _D), _F32),
            pltpu.VMEM((_B, _H, _DC), _F32),
            pltpu.VMEM((_H, 128), _F32),
            pltpu.VMEM((_H, 128), _F32),
            pltpu.VMEM((_H, _DC), _F32),
            pltpu.VMEM((_H, 8, _DC), _F32),
            pltpu.VMEM((_H, 8, _D), _F32),
            pltpu.VMEM((_B * _H, _D), _F32),
            pltpu.VMEM((_B, 8, _M), _F32),
            dma((2,)), dma((_B,)), dma((5,)), dma((_NC,)), dma((_NSLOT,)), dma((_NSLOT,)),
        ],
        compiler_params=pltpu.CompilerParams(vmem_limit_bytes=100 * 1024 * 1024),
    )(
        A_x.reshape(_B, _M),
        A_c_kv.reshape((_B,) + wide_w),
        A_w_q.reshape(head_w),
        A_w_uk.reshape(head_w),
        A_w_uv.reshape(head_w),
        A_w_o.reshape(wide_w),
        B_x.reshape(_B, _M),
        B_k_cache.reshape(_B * _H, _SK, _D),
        B_v_cache.reshape(_B * _H, _SK, _D),
        B_wq.reshape(wqb_w),
        B_wo.reshape(wide_w),
    )
    return out.reshape(_B, 1, 2 * _M)
```

```python
import jax
import jax.numpy as jnp
from jax import lax
import jax.experimental.pallas as pl
import jax.experimental.pallas.tpu as pltpu

_B, _H, _D, _SK, _M, _DC = 4, 32, 128, 4096, 512, 512
_HG = 8
_NC = 8
_RC = _SK // _NC
_NG = _B * _H // _HG
_NSLOT = 4
_AHEAD = 2
_KV = 32
_UNIT = 128
_SHARE = _UNIT // _NC

_F32 = jnp.float32
_BF16 = jnp.bfloat16
_U32 = jnp.uint32


def _dot(a, b):
    return jnp.dot(a, b, preferred_element_type=_F32)


def _dot_nt(a, b):
    return lax.dot_general(a, b, (((1,), (1,)), ((), ())), preferred_element_type=_F32)


def _ds(start, size):
    return pl.ds(start if isinstance(start, int) else pl.multiple_of(start, size), size)


def _lane_sum(x):
    return sum(x[:, t:t + 128] for t in range(0, x.shape[1], 128))


def _kernel(xa_hbm, c_hbm, wqa_hbm, wuk_hbm, wuv_hbm, woa_hbm,
            xb_hbm, k_hbm, v_hbm, wqb_hbm, wob_hbm,
            o_ref,
            xa_buf, c_buf, wqa_buf, wuk_buf, wuv_buf, woa_buf,
            xb_buf, kv_buf, wqb_buf, wob_buf,
            words_s, xa_s, qa_s, qabs_s, ma_s, la_s, acca_s, cl_s, ctx_s, qb_s, outb_s,
            x_sem, c_sem, w_sem, woa_sem, k_sem, v_sem):
    scale = _D ** -0.5
    k_buf, v_buf = kv_buf.at[0], kv_buf.at[1]

    wqb, wob, wqa, wuk, wuv = (
        (src, dst, w_sem.at[i]) for i, (src, dst) in enumerate((
            (wqb_hbm, wqb_buf), (wob_hbm, wob_buf),
            (wqa_hbm, wqa_buf), (wuk_hbm, wuk_buf), (wuv_hbm, wuv_buf))))

    def latent(b):
        return c_hbm.at[b], c_buf.at[b], c_sem.at[b]

    def start_unit(unit, share, t, queue):
        src, dst, sem = unit
        n = src.shape[1] * 2 // _UNIT
        at = (pl.ds(t % 2 * 2, 2), _ds((share * (_SHARE // 2) + t // 2) * n, n))
        pltpu.make_async_copy(src.at[at], dst.at[at], sem).start(priority=queue)

    def start_kv(step, j):
        slot = step % _NSLOT
        head, row = j % 4 * 2, j // 4 * 64
        src = (_ds(step // _NC * _HG + head, 2), _ds(step % _NC * _RC + row, 64))
        dst = (slot, pl.ds(head, 2), pl.ds(row, 64))
        pltpu.make_async_copy(k_hbm.at[src], k_buf.at[dst], k_sem.at[slot]).start(priority=1)
        pltpu.make_async_copy(v_hbm.at[src], v_buf.at[dst], v_sem.at[slot]).start(priority=0)

    def wait_all(buf, sem):
        pltpu.make_async_copy(buf, buf, sem).wait()

    def heads_of(buf, c):
        first = c % 2 * (_H // 2)
        block = buf[c // 2, :, _ds(first, _H // 2), :].reshape(128 * _H // 2, _D)
        words_s[...] = pltpu.bitcast(block, _U32)
        for j in range(_H // 4):
            words = words_s[pl.ds(j, 128, stride=_H // 4), :]
            even = lax.bitcast_convert_type(words << 16, _F32)
            odd = lax.bitcast_convert_type(words & jnp.uint32(0xFFFF0000), _F32)
            yield first + 2 * j, even.astype(_BF16)
            yield first + 2 * j + 1, odd.astype(_BF16)

    def rows8(x_buf):
        x = x_buf[...].astype(_F32)
        return jnp.concatenate([x, jnp.zeros_like(x)], axis=0)

    def a_query(c):
        x = xa_s[c // 2].astype(_BF16)
        for h, w in heads_of(wqa_buf, c):
            qa_s[h] += _dot(x, w)

    def a_absorb(c):
        for h, w in heads_of(wuk_buf, c):
            qabs = _dot_nt(qa_s[h].astype(_BF16), w)
            for b in range(_B):
                qabs_s[b, c // 2, pl.ds(h, 1), :] = qabs[b:b + 1]

    def a_attend(b, c):
        @pl.when(c == 0)
        def _():
            ma_s[...] = jnp.full(ma_s.shape, -jnp.inf, _F32)
            la_s[...] = jnp.zeros(la_s.shape, _F32)
            acca_s[...] = jnp.zeros(acca_s.shape, _F32)

        lat = c_buf[b, c // 2, _ds(c % 2 * _RC, _RC), :]
        qabs = jnp.concatenate([qabs_s[b, i] for i in range(_DC // 128)], axis=1)
        s = _dot_nt(qabs.astype(_BF16), lat) * scale
        m_old = ma_s[...]
        m_new = jnp.maximum(m_old, jnp.max(s, axis=1, keepdims=True))
        alpha = jnp.exp(m_old - m_new)
        p = jnp.exp(s - m_new[:, :1])
        ma_s[...] = m_new
        la_s[...] = alpha * la_s[...] + _lane_sum(p)
        acca_s[...] = alpha[:, :1] * acca_s[...] + _dot(p.astype(_BF16), lat)

        @pl.when(c == _NC - 1)
        def _():
            ctx = acca_s[...] / jnp.sum(la_s[...], axis=1, keepdims=True)
            for i in range(_DC // 128):
                for h in range(_H):
                    cl_s[i, h, pl.ds(b, 1), :] = ctx[h:h + 1, i * 128:(i + 1) * 128]

    def a_value(c):
        for h, w in heads_of(wuv_buf, c):
            ctx_s[h] += _dot(cl_s[c // 2, h].astype(_BF16), w)

    def a_output(c):
        share = woa_buf.at[:, pl.ds(c * _D, _D)]
        wait_all(share, woa_sem.at[c])
        ctx = jnp.concatenate([ctx_s[h] for h in range(c, _H, _NC)], axis=1)
        return _dot(ctx.astype(_BF16), share[...].reshape(_H // _NC * _D, _M))

    def side_work(g, c):
        def fetch(*units):
            for t in range(_SHARE):
                for queue, unit in enumerate(units):
                    start_unit(unit, c, t, queue)

        def consume(unit, work):
            pl.when(c == 0)(lambda: wait_all(*unit[1:]))
            work(c)

        pl.when(g == 0)(lambda: fetch(wob, wqa))
        pl.when(g == 1)(lambda: fetch(wuk, wuv))
        pl.when((g >= 2) & (g < 2 + _B // 2))(
            lambda: fetch(latent(g - 2), latent(g - 2 + _B // 2)))
        pl.when(g == 1)(lambda: consume(wqa, a_query))
        pl.when(g == 2)(lambda: consume(wuk, a_absorb))
        pl.when((g >= 3) & (g < 3 + _B))(
            lambda: consume(latent(g - 3), lambda c: a_attend(g - 3, c)))
        pl.when(g == 3 + _B)(lambda: consume(wuv, a_value))

    def start_wqb(i):
        for t in range(_SHARE):
            at = (pl.ds(t % 2 * 2, 2), _ds((i * 2 + t // 8) * 8, 8), pl.ds(t // 2 % 4 * 1024, 1024))
            pltpu.make_async_copy(wqb_hbm.at[at], wqb_buf.at[at], wqb[2]).start(priority=t % 2)

    xb_copy = pltpu.make_async_copy(xb_hbm, xb_buf, x_sem.at[0])
    xa_copy = pltpu.make_async_copy(xa_hbm, xa_buf, x_sem.at[1])
    start_wqb(0)
    xb_copy.start()
    xa_copy.start()
    pl.loop(1, _NC)(start_wqb)
    for step in range(_AHEAD - 1):
        for j in range(_KV):
            start_kv(step, j)

    for ref in (qa_s, cl_s, ctx_s, outb_s):
        ref[...] = jnp.zeros(ref.shape, _F32)

    xb_copy.wait()
    xa_copy.wait()
    xb = rows8(xb_buf).astype(_BF16)
    xa = rows8(xa_buf)
    for i in range(_M // 128):
        xa_s[i] = xa[:, i * 128:(i + 1) * 128]
    wait_all(*wqb[1:])
    for h in range(_H):
        q = _dot(xb, wqb_buf[:, :, h * _D:(h + 1) * _D].reshape(_M, _D))
        for b in range(_B):
            qb_s[pl.ds(b * _H + h, 1), :] = q[b:b + 1]
        start_kv(_AHEAD - 1, h)

    sub = lax.broadcasted_iota(jnp.int32, (_HG, _D), 0)
    sub_rc = lax.broadcasted_iota(jnp.int32, (_HG, _RC), 0)
    n_dot = 2 * _HG

    def request_kv(step):
        def request(i):
            for j in range(i * _KV // n_dot, (i + 1) * _KV // n_dot):
                start_kv(step, j)
        return request

    def request_woa(part):
        def request(i):
            n = _UNIT // (_AHEAD * n_dot)
            for j in range((part * n_dot + i) * n, (part * n_dot + i + 1) * n):
                share = j // _SHARE
                start_unit((woa_hbm, woa_buf, woa_sem.at[share]), share, j % _SHARE, j % 2)
        return request

    def kv_step(step, q, carry, request):
        m, l, acc = carry
        slot = step % _NSLOT
        wait_all(k_buf.at[slot], k_sem.at[slot])
        s = None
        for i in range(_HG):
            si = _dot_nt(q, k_buf[slot, i])
            s = si if s is None else jnp.where(sub_rc == i, si, s)
            request(i)
        s = s * scale
        m_new = jnp.maximum(m, jnp.max(s, axis=1, keepdims=True))
        alpha = jnp.exp(m - m_new)
        p = jnp.exp(s - m_new)
        l = alpha * l + _lane_sum(p)
        p = p.astype(_BF16)
        wait_all(v_buf.at[slot], v_sem.at[slot])
        pv = None
        for i in range(_HG):
            pvi = _dot(p, v_buf[slot, i])
            pv = pvi if pv is None else jnp.where(sub == i, pvi, pv)
            request(_HG + i)
        return m_new, l, alpha * acc + pv

    def group(g, last):
        q = qb_s[_ds(g * _HG, _HG), :].astype(_BF16)
        carry = (jnp.full((_HG, 1), -jnp.inf, _F32), jnp.zeros((_HG, _D), _F32),
                 jnp.zeros((_HG, _D), _F32))

        def body(c, carry):
            if not last:
                pl.when(g <= 3 + _B)(lambda: side_work(g, c))
            step = g * _NC + c
            return kv_step(step, q, carry, request_kv(step + _AHEAD))

        if last:
            carry = lax.fori_loop(0, _NC - _AHEAD, body, carry)
            for part in range(_AHEAD):
                carry = kv_step((g + 1) * _NC - _AHEAD + part, q, carry, request_woa(part))
        else:
            carry = lax.fori_loop(0, _NC, body, carry)
            pl.when(g == 0)(lambda: wait_all(*wob[1:]))
        _, l, acc = carry
        o = acc / jnp.sum(l, axis=1, keepdims=True)
        o = jnp.concatenate([jnp.where(sub == i, o, 0.0) for i in range(_HG)], axis=1)
        outb_s[g // (_H // _HG)] += _dot(o.astype(_BF16), wob_buf[g % (_H // _HG)])

    pl.loop(0, _NG - 1)(lambda g: group(g, False))
    group(_NG - 1, True)

    out_b = jnp.concatenate(
        [jnp.sum(outb_s[b], axis=0, keepdims=True) for b in range(_B)], axis=0)
    o_ref[:, _M:2 * _M] = out_b.astype(o_ref.dtype)
    out_a = sum(a_output(c) for c in range(_NC))
    o_ref[:, 0:_M] = out_a[0:_B].astype(o_ref.dtype)


@jax.jit
def pallas_concat_heads__compressed_kv_cla__mha_block_cached__decode_kernel(
    A_x: jax.Array,
    A_c_kv: jax.Array,
    A_w_q: jax.Array,
    A_w_uk: jax.Array,
    A_w_uv: jax.Array,
    A_w_o: jax.Array,
    B_x: jax.Array,
    B_k_cache: jax.Array,
    B_v_cache: jax.Array,
    B_wq: jax.Array,
    B_wo: jax.Array,
):
    assert A_x.shape == B_x.shape == (_B, 1, _M) and A_c_kv.shape == (_B, _SK, _DC)
    assert A_w_q.shape == (_M, _H, _D) and B_k_cache.shape == (_B, _H, _SK, _D)
    head_w = (4, _M // 4, _H, _D)
    wide_w = (4, _SK // 4, _DC)
    wqb_w = (4, _M // 4, _H * _D)
    dma = pltpu.SemaphoreType.DMA
    out = pl.pallas_call(
        _kernel,
        in_specs=[pl.BlockSpec(memory_space=pl.ANY)] * 11,
        out_specs=pl.BlockSpec(memory_space=pltpu.VMEM),
        out_shape=jax.ShapeDtypeStruct((_B, 2 * _M), A_x.dtype),
        scratch_shapes=[
            pltpu.VMEM((_B, _M), _BF16),
            pltpu.VMEM((_B,) + wide_w, _BF16),
            pltpu.VMEM(head_w, _BF16),
            pltpu.VMEM(head_w, _BF16),
            pltpu.VMEM(head_w, _BF16),
            pltpu.VMEM(wide_w, _BF16),
            pltpu.VMEM((_B, _M), _BF16),
            pltpu.VMEM((2, _NSLOT, _HG, _RC, _D), _BF16),
            pltpu.VMEM(wqb_w, _BF16),
            pltpu.VMEM(wide_w, _BF16),
            pltpu.VMEM((128 * _H // 4, _D), _U32),
            pltpu.VMEM((_M // 128, 8, 128), _F32),
            pltpu.VMEM((_H, 8, _D), _F32),
            pltpu.VMEM((_B, _DC // 128, _H, 128), _F32),
            pltpu.VMEM((_H, 128), _F32),
            pltpu.VMEM((_H, 128), _F32),
            pltpu.VMEM((_H, _DC), _F32),
            pltpu.VMEM((_DC // 128, _H, 8, 128), _F32),
            pltpu.VMEM((_H, 8, _D), _F32),
            pltpu.VMEM((_B * _H, _D), _F32),
            pltpu.VMEM((_B, 8, _M), _F32),
            dma((2,)), dma((_B,)), dma((5,)), dma((_NC,)), dma((_NSLOT,)), dma((_NSLOT,)),
        ],
        compiler_params=pltpu.CompilerParams(vmem_limit_bytes=100 * 1024 * 1024),
    )(
        A_x.reshape(_B, _M),
        A_c_kv.reshape((_B,) + wide_w),
        A_w_q.reshape(head_w),
        A_w_uk.reshape(head_w),
        A_w_uv.reshape(head_w),
        A_w_o.reshape(wide_w),
        B_x.reshape(_B, _M),
        B_k_cache.reshape(_B * _H, _SK, _D),
        B_v_cache.reshape(_B * _H, _SK, _D),
        B_wq.reshape(wqb_w),
        B_wo.reshape(wide_w),
    )
    return out.reshape(_B, 1, 2 * _M)
```

```python
import jax
import jax.numpy as jnp
from jax import lax
import jax.experimental.pallas as pl
import jax.experimental.pallas.tpu as pltpu

_B, _H, _D, _SK, _M, _DC = 4, 32, 128, 4096, 512, 512
_HG = 8
_NC = 8
_RC = _SK // _NC
_NG = _B * _H // _HG
_NSLOT = 4
_AHEAD = 2
_KV = 32
_UNIT = 128
_SHARE = _UNIT // _NC

_F32 = jnp.float32
_BF16 = jnp.bfloat16
_U32 = jnp.uint32
_LOWEST = -3.4028234663852886e38


def _dot(a, b):
    return jnp.dot(a, b, preferred_element_type=_F32)


def _dot_nt(a, b):
    return lax.dot_general(a, b, (((1,), (1,)), ((), ())), preferred_element_type=_F32)


def _ds(start, size):
    return pl.ds(start if isinstance(start, int) else pl.multiple_of(start, size), size)


def _lane_sum(x):
    return sum(x[:, t:t + 128] for t in range(0, x.shape[1], 128))


def _kernel(xa_hbm, c_hbm, wqa_hbm, wuk_hbm, wuv_hbm, woa_hbm,
            xb_hbm, k_hbm, v_hbm, wqb_hbm, wob_hbm,
            o_ref,
            xa_buf, c_buf, wqa_buf, wuk_buf, wuv_buf, woa_buf,
            xb_buf, kv_buf, wqb_buf, wob_buf,
            words_s, xa_s, qa_s, qabs_s, ma_s, la_s, acca_s, cl_s, ctx_s, qb_s, outb_s,
            x_sem, c_sem, w_sem, woa_sem, k_sem, v_sem):
    scale = _D ** -0.5
    k_buf, v_buf = kv_buf.at[0], kv_buf.at[1]

    wqb, wob, wqa, wuk, wuv = (
        (src, dst, w_sem.at[i]) for i, (src, dst) in enumerate((
            (wqb_hbm, wqb_buf), (wob_hbm, wob_buf),
            (wqa_hbm, wqa_buf), (wuk_hbm, wuk_buf), (wuv_hbm, wuv_buf))))

    def latent(b):
        return c_hbm.at[b], c_buf.at[b], c_sem.at[b]

    def start_unit(unit, share, t, queue):
        src, dst, sem = unit
        n = src.shape[1] * 2 // _UNIT
        at = (pl.ds(t % 2 * 2, 2), _ds((share * (_SHARE // 2) + t // 2) * n, n))
        pltpu.make_async_copy(src.at[at], dst.at[at], sem).start(priority=queue)

    def start_kv(step, j):
        slot = step % _NSLOT
        head, row = j % 4 * 2, j // 4 * 64
        src = (_ds(step // _NC * _HG + head, 2), _ds(step % _NC * _RC + row, 64))
        dst = (slot, pl.ds(head, 2), pl.ds(row, 64))
        pltpu.make_async_copy(k_hbm.at[src], k_buf.at[dst], k_sem.at[slot]).start(priority=1)
        pltpu.make_async_copy(v_hbm.at[src], v_buf.at[dst], v_sem.at[slot]).start(priority=0)

    def wait_all(buf, sem):
        pltpu.make_async_copy(buf, buf, sem).wait()

    def heads_of(buf, c):
        first = c % 2 * (_H // 2)
        block = buf[c // 2, :, _ds(first, _H // 2), :].reshape(128 * _H // 2, _D)
        words_s[...] = pltpu.bitcast(block, _U32)
        for j in range(_H // 4):
            words = words_s[pl.ds(j, 128, stride=_H // 4), :]
            even = lax.bitcast_convert_type(words << 16, _F32)
            odd = lax.bitcast_convert_type(words & jnp.uint32(0xFFFF0000), _F32)
            yield first + 2 * j, even.astype(_BF16)
            yield first + 2 * j + 1, odd.astype(_BF16)

    def rows8(x_buf):
        x = x_buf[...].astype(_F32)
        return jnp.concatenate([x, jnp.zeros_like(x)], axis=0)

    def a_query(c):
        x = xa_s[c // 2].astype(_BF16)
        for h, w in heads_of(wqa_buf, c):
            qa_s[h] += _dot(x, w)

    def a_absorb(c):
        for h, w in heads_of(wuk_buf, c):
            qabs = _dot_nt(qa_s[h].astype(_BF16), w)
            for b in range(_B):
                qabs_s[b, c // 2, pl.ds(h, 1), :] = qabs[b:b + 1]

    def a_attend(b, c):
        @pl.when(c == 0)
        def _():
            ma_s[...] = jnp.full(ma_s.shape, _LOWEST, _F32)
            la_s[...] = jnp.zeros(la_s.shape, _F32)
            acca_s[...] = jnp.zeros(acca_s.shape, _F32)

        lat = c_buf[b, c // 2, _ds(c % 2 * _RC, _RC), :]
        qabs = jnp.concatenate([qabs_s[b, i] for i in range(_DC // 128)], axis=1)
        s = _dot_nt(qabs.astype(_BF16), lat) * scale
        m_old = ma_s[...]
        m_new = jnp.maximum(m_old, jnp.max(s, axis=1, keepdims=True))
        alpha = jnp.exp(m_old - m_new)
        p = jnp.exp(s - m_new[:, :1])
        ma_s[...] = m_new
        la_s[...] = alpha * la_s[...] + _lane_sum(p)
        acca_s[...] = alpha[:, :1] * acca_s[...] + _dot(p.astype(_BF16), lat)

        @pl.when(c == _NC - 1)
        def _():
            ctx = acca_s[...] / jnp.sum(la_s[...], axis=1, keepdims=True)
            for i in range(_DC // 128):
                for h in range(_H):
                    cl_s[i, h, pl.ds(b, 1), :] = ctx[h:h + 1, i * 128:(i + 1) * 128]

    def a_value(c):
        for h, w in heads_of(wuv_buf, c):
            ctx_s[h] += _dot(cl_s[c // 2, h].astype(_BF16), w)

    def a_output(c):
        share = woa_buf.at[:, pl.ds(c * _D, _D)]
        wait_all(share, woa_sem.at[c])
        ctx = jnp.concatenate([ctx_s[h] for h in range(c, _H, _NC)], axis=1)
        return _dot(ctx.astype(_BF16), share[...].reshape(_H // _NC * _D, _M))

    def side_work(g, c):
        def fetch(*units):
            for t in range(_SHARE):
                for queue, unit in enumerate(units):
                    start_unit(unit, c, t, queue)

        def consume(unit, work):
            pl.when(c == 0)(lambda: wait_all(*unit[1:]))
            work(c)

        pl.when(g == 0)(lambda: fetch(wob, wqa))
        pl.when(g == 1)(lambda: fetch(wuk, wuv))
        pl.when((g >= 2) & (g < 2 + _B // 2))(
            lambda: fetch(latent(g - 2), latent(g - 2 + _B // 2)))
        pl.when(g == 1)(lambda: consume(wqa, a_query))
        pl.when(g == 2)(lambda: consume(wuk, a_absorb))
        pl.when((g >= 3) & (g < 3 + _B))(
            lambda: consume(latent(g - 3), lambda c: a_attend(g - 3, c)))
        pl.when(g == 3 + _B)(lambda: consume(wuv, a_value))

    def start_wqb(i):
        for t in range(_SHARE):
            at = (pl.ds(t % 2 * 2, 2), _ds((i * 2 + t // 8) * 8, 8), pl.ds(t // 2 % 4 * 1024, 1024))
            pltpu.make_async_copy(wqb_hbm.at[at], wqb_buf.at[at], wqb[2]).start(priority=t % 2)

    xb_copy = pltpu.make_async_copy(xb_hbm, xb_buf, x_sem.at[0])
    xa_copy = pltpu.make_async_copy(xa_hbm, xa_buf, x_sem.at[1])
    start_wqb(0)
    xb_copy.start()
    xa_copy.start()
    pl.loop(1, _NC)(start_wqb)
    for step in range(_AHEAD - 1):
        for j in range(_KV):
            start_kv(step, j)

    for ref in (qa_s, cl_s, ctx_s, outb_s):
        ref[...] = jnp.zeros(ref.shape, _F32)

    xb_copy.wait()
    xa_copy.wait()
    xb = rows8(xb_buf).astype(_BF16)
    xa = rows8(xa_buf)
    for i in range(_M // 128):
        xa_s[i] = xa[:, i * 128:(i + 1) * 128]
    wait_all(*wqb[1:])
    for h in range(_H):
        q = _dot(xb, wqb_buf[:, :, h * _D:(h + 1) * _D].reshape(_M, _D))
        for b in range(_B):
            qb_s[pl.ds(b * _H + h, 1), :] = q[b:b + 1]
        start_kv(_AHEAD - 1, h)

    sub = lax.broadcasted_iota(jnp.int32, (_HG, _D), 0)
    sub_rc = lax.broadcasted_iota(jnp.int32, (_HG, _RC), 0)
    n_dot = 2 * _HG

    def request_kv(step):
        def request(i):
            for j in range(i * _KV // n_dot, (i + 1) * _KV // n_dot):
                start_kv(step, j)
        return request

    def request_woa(part):
        def request(i):
            n = _UNIT // (_AHEAD * n_dot)
            for j in range((part * n_dot + i) * n, (part * n_dot + i + 1) * n):
                share = j // _SHARE
                start_unit((woa_hbm, woa_buf, woa_sem.at[share]), share, j % _SHARE, j % 2)
        return request

    def kv_step(step, q, carry, request):
        m, l, acc = carry
        slot = step % _NSLOT
        wait_all(k_buf.at[slot], k_sem.at[slot])
        s = None
        for i in range(_HG):
            si = _dot_nt(q, k_buf[slot, i])
            s = si if s is None else jnp.where(sub_rc == i, si, s)
            request(i)
        s = s * scale
        m_new = jnp.maximum(m, jnp.max(s, axis=1, keepdims=True))
        alpha = jnp.exp(m - m_new)
        p = jnp.exp(s - m_new)
        l = alpha * l + _lane_sum(p)
        p = p.astype(_BF16)
        wait_all(v_buf.at[slot], v_sem.at[slot])
        pv = None
        for i in range(_HG):
            pvi = _dot(p, v_buf[slot, i])
            pv = pvi if pv is None else jnp.where(sub == i, pvi, pv)
            request(_HG + i)
        return m_new, l, alpha * acc + pv

    def group(g, last):
        q = qb_s[_ds(g * _HG, _HG), :].astype(_BF16)
        carry = (jnp.full((_HG, 1), _LOWEST, _F32), jnp.zeros((_HG, _D), _F32),
                 jnp.zeros((_HG, _D), _F32))

        def body(c, carry):
            if not last:
                pl.when(g <= 3 + _B)(lambda: side_work(g, c))
            step = g * _NC + c
            return kv_step(step, q, carry, request_kv(step + _AHEAD))

        if last:
            carry = lax.fori_loop(0, _NC - _AHEAD, body, carry)
            for part in range(_AHEAD):
                carry = kv_step((g + 1) * _NC - _AHEAD + part, q, carry, request_woa(part))
        else:
            carry = lax.fori_loop(0, _NC, body, carry)
            pl.when(g == 0)(lambda: wait_all(*wob[1:]))
        _, l, acc = carry
        o = acc / jnp.sum(l, axis=1, keepdims=True)
        o = jnp.concatenate([jnp.where(sub == i, o, 0.0) for i in range(_HG)], axis=1)
        outb_s[g // (_H // _HG)] += _dot(o.astype(_BF16), wob_buf[g % (_H // _HG)])

    pl.loop(0, _NG - 1)(lambda g: group(g, False))
    group(_NG - 1, True)

    out_b = jnp.concatenate(
        [jnp.sum(outb_s[b], axis=0, keepdims=True) for b in range(_B)], axis=0)
    o_ref[:, _M:2 * _M] = out_b.astype(o_ref.dtype)
    out_a = sum(a_output(c) for c in range(_NC))
    o_ref[:, 0:_M] = out_a[0:_B].astype(o_ref.dtype)


@jax.jit
def pallas_concat_heads__compressed_kv_cla__mha_block_cached__decode_kernel(
    A_x: jax.Array,
    A_c_kv: jax.Array,
    A_w_q: jax.Array,
    A_w_uk: jax.Array,
    A_w_uv: jax.Array,
    A_w_o: jax.Array,
    B_x: jax.Array,
    B_k_cache: jax.Array,
    B_v_cache: jax.Array,
    B_wq: jax.Array,
    B_wo: jax.Array,
):
    assert A_x.shape == B_x.shape == (_B, 1, _M) and A_c_kv.shape == (_B, _SK, _DC)
    assert A_w_q.shape == (_M, _H, _D) and B_k_cache.shape == (_B, _H, _SK, _D)
    head_w = (4, _M // 4, _H, _D)
    wide_w = (4, _SK // 4, _DC)
    wqb_w = (4, _M // 4, _H * _D)
    dma = pltpu.SemaphoreType.DMA
    out = pl.pallas_call(
        _kernel,
        in_specs=[pl.BlockSpec(memory_space=pl.ANY)] * 11,
        out_specs=pl.BlockSpec(memory_space=pltpu.VMEM),
        out_shape=jax.ShapeDtypeStruct((_B, 2 * _M), A_x.dtype),
        scratch_shapes=[
            pltpu.VMEM((_B, _M), _BF16),
            pltpu.VMEM((_B,) + wide_w, _BF16),
            pltpu.VMEM(head_w, _BF16),
            pltpu.VMEM(head_w, _BF16),
            pltpu.VMEM(head_w, _BF16),
            pltpu.VMEM(wide_w, _BF16),
            pltpu.VMEM((_B, _M), _BF16),
            pltpu.VMEM((2, _NSLOT, _HG, _RC, _D), _BF16),
            pltpu.VMEM(wqb_w, _BF16),
            pltpu.VMEM(wide_w, _BF16),
            pltpu.VMEM((128 * _H // 4, _D), _U32),
            pltpu.VMEM((_M // 128, 8, 128), _F32),
            pltpu.VMEM((_H, 8, _D), _F32),
            pltpu.VMEM((_B, _DC // 128, _H, 128), _F32),
            pltpu.VMEM((_H, 128), _F32),
            pltpu.VMEM((_H, 128), _F32),
            pltpu.VMEM((_H, _DC), _F32),
            pltpu.VMEM((_DC // 128, _H, 8, 128), _F32),
            pltpu.VMEM((_H, 8, _D), _F32),
            pltpu.VMEM((_B * _H, _D), _F32),
            pltpu.VMEM((_B, 8, _M), _F32),
            dma((2,)), dma((_B,)), dma((5,)), dma((_NC,)), dma((_NSLOT,)), dma((_NSLOT,)),
        ],
        compiler_params=pltpu.CompilerParams(vmem_limit_bytes=64 * 1024 * 1024),
    )(
        A_x.reshape(_B, _M),
        A_c_kv.reshape((_B,) + wide_w),
        A_w_q.reshape(head_w),
        A_w_uk.reshape(head_w),
        A_w_uv.reshape(head_w),
        A_w_o.reshape(wide_w),
        B_x.reshape(_B, _M),
        B_k_cache.reshape(_B * _H, _SK, _D),
        B_v_cache.reshape(_B * _H, _SK, _D),
        B_wq.reshape(wqb_w),
        B_wo.reshape(wide_w),
    )
    return out.reshape(_B, 1, 2 * _M)
```
